```python
import os as _os
_os.environ.setdefault("JAX_PLATFORMS", "cpu")
import jax
import jax.numpy as jnp

def _softmax(x, axis=-1):
    return jax.nn.softmax(x, axis=axis)
def _gelu(x):
    return jax.nn.gelu(x, approximate=True)
def _silu(x):
    return jax.nn.silu(x)
def _sigmoid(x):
    return jax.nn.sigmoid(x)
def _layernorm(x, axis=-1, eps=1e-5):
    m = jnp.mean(x, axis=axis, keepdims=True)
    v = jnp.var(x, axis=axis, keepdims=True)
    return (x - m) / jnp.sqrt(v + eps)
def _scatter_add(tgt, idx, src, axis=0):
    return tgt.at[idx].add(src)
def _segment_sum(src, seg, n):
    return jax.ops.segment_sum(src, seg, n)
class _Rng:
    def __init__(self, key):
        self._k = key
    def _next(self):
        self._k, sub = jax.random.split(self._k)
        return sub
    def normal(self, shape):
        return jax.random.normal(self._next(), shape, dtype=jnp.bfloat16)
    def randint(self, lo, hi, shape):
        return jax.random.randint(self._next(), shape, lo, hi, dtype=jnp.int32)
    def uniform(self, shape, lo=0.0, hi=1.0):
        return jax.random.uniform(self._next(), shape, jnp.bfloat16, lo, hi)
    def permutation(self, n):
        return jax.random.permutation(self._next(), n)


kernel_name = 'standalone__mha_softmax__near_ridge'

def setup_inputs():
    _rng = _Rng(jax.random.key(int.from_bytes(__import__("os").urandom(4), "little")))
    _w = (lambda a: (lambda t: t.astype(jnp.bfloat16) if jnp.issubdtype(t.dtype, jnp.floating) else t)(jnp.asarray(a)))
    B, H, Sq, Sk, D = 8, 32, 496, 512, 192
    return {
        "q": _w((lambda *s: _rng.normal(s) * 0.05)(B, H, Sq, D)),
        "k": _w((lambda *s: _rng.normal(s) * 3.2)(B, H, Sk, D)),
        "v": _w((lambda *s: _rng.normal(s) * 0.05)(B, H, Sk, D)),
    }

def reference(q, k, v):
    scale = q.shape[-1] ** -0.5
    scores = jnp.einsum("bhqd,bhkd->bhqk", q, k) * scale
    p = _softmax(scores, axis=-1)
    return jnp.einsum("bhqk,bhkd->bhqd", p, v)
```

```python
import functools
import math

import jax
import jax.numpy as jnp
from jax import lax
import jax.experimental.pallas as pl
import jax.experimental.pallas.tpu as pltpu

_HB = 8
_SPLITS = ((0, 256), (256, 496))
_LOOK = 2
_FLAGS = {"XLA_TPU_FORCE_LP_LLO_SCHEDULER": True}
_KT_AHEAD = 0


def _mha_kernel(qt_ref, kt_ref, vt_ref, ot_ref, *, scale, hb):
    c = scale * math.log2(math.e)
    units = [(h, c0, c1) for h in range(hb) for (c0, c1) in _SPLITS]
    n = len(units)
    kts = {}
    S = {}
    P = {}

    def KT(h):
        if h < hb and h not in kts:
            kts[h] = kt_ref[h].T

    def QK(i):
        h, c0, c1 = units[i]
        KT(h)
        for a in range(1, _KT_AHEAD + 1):
            KT(h + a)
        S[i] = jnp.dot(kts[h], qt_ref[h, :, c0:c1], preferred_element_type=jnp.float32)

    def SM(i):
        s = S.pop(i)
        m = jnp.max(s, axis=0, keepdims=True)
        p = jnp.exp2((s - m) * c)
        l = jnp.sum(p, axis=0, keepdims=True)
        P[i] = (p.astype(jnp.bfloat16), l)

    def PV(i):
        h, c0, c1 = units[i]
        p, l = P.pop(i)
        o = jnp.dot(vt_ref[h], p, preferred_element_type=jnp.float32)
        ot_ref[h, :, c0:c1] = (o * (1.0 / l)).astype(ot_ref.dtype)

    for i in range(min(_LOOK, n)):
        QK(i)
    for i in range(n):
        if i + _LOOK < n:
            QK(i + _LOOK)
        SM(i)
        PV(i)


@jax.jit
def pallas_standalone__mha_softmax__near_ridge_kernel(q, k, v):
    B, H, Sq, D = q.shape
    Sk = k.shape[2]
    scale = float(D) ** -0.5
    qt = jnp.swapaxes(q, 2, 3).reshape(B * H, D, Sq)
    kt = jnp.swapaxes(k, 2, 3).reshape(B * H, D, Sk)
    vt = jnp.swapaxes(v, 2, 3).reshape(B * H, D, Sk)
    hb = _HB
    ot = pl.pallas_call(
        functools.partial(_mha_kernel, scale=scale, hb=hb),
        grid=(B * H // hb,),
        in_specs=[
            pl.BlockSpec((hb, D, Sq), lambda i: (i, 0, 0)),
            pl.BlockSpec((hb, D, Sk), lambda i: (i, 0, 0)),
            pl.BlockSpec((hb, D, Sk), lambda i: (i, 0, 0)),
        ],
        out_specs=pl.BlockSpec((hb, D, Sq), lambda i: (i, 0, 0)),
        out_shape=jax.ShapeDtypeStruct((B * H, D, Sq), q.dtype),
        compiler_params=pltpu.CompilerParams(
            dimension_semantics=("parallel",),
            vmem_limit_bytes=64 * 1024 * 1024,
            flags=_FLAGS,
        ),
    )(qt, kt, vt)
    return jnp.swapaxes(ot.reshape(B, H, D, Sq), 2, 3)
```

```python
import functools
import math

import jax
import jax.numpy as jnp
from jax import lax
import jax.experimental.pallas as pl
import jax.experimental.pallas.tpu as pltpu

_G = 8
_RAMP_IN = (1, 1, 2, 4)
_RAMP_OUT = (4, 2, 1, 1)
_FLAGS = None
_CH = 128
_ORDER = 'headlook'
_CARRY = True
_PAD = True
_LAZY_L = True


def _compute_heads(heads, get_kt, emit_kt_next, qb, vb, ob, slot, c):
    Sq = qb.shape[-1]
    W = 256
    splits = [(c0, min(c0 + W, Sq)) for c0 in range(0, Sq, W)]
    nsp = len(splits)
    S = {}
    P = {}

    def QK(j, u):
        c0, c1 = splits[u]
        qq = qb[slot, j, :, c0:c1]
        if _PAD and c1 - c0 < W:
            qq = jnp.pad(qq, ((0, 0), (0, W - (c1 - c0))))
        S[j, u] = jnp.dot(get_kt(j), qq, preferred_element_type=jnp.float32)

    def SM(j, u):
        s = S.pop((j, u))
        nch = s.shape[0] // _CH
        w = s.shape[1]
        ms, ps, ls = [], [], []
        m = None
        for t in range(nch):
            st = s[t * _CH:(t + 1) * _CH] * c
            mt = jnp.max(st, axis=0, keepdims=True)
            m = mt if m is None else jnp.maximum(m, mt)
            p = jnp.exp2(st - m)
            ms.append(m)
            if _LAZY_L:
                ls.append(jnp.sum(p.reshape(_CH // 8, 8, w), axis=0))
            else:
                ls.append(jnp.sum(p, axis=0, keepdims=True))
            ps.append(p.astype(jnp.bfloat16))
        al = [jnp.exp2(mm - m) for mm in ms[:-1]]
        l = ls[-1]
        for t in range(nch - 1):
            l = l + al[t] * ls[t]
        if _LAZY_L:
            l = jnp.sum(l, axis=0, keepdims=True)
        r = 1.0 / l
        P[j, u] = (ps, [a * r for a in al] + [r])

    def PV(j, u):
        c0, c1 = splits[u]
        ps, be = P.pop((j, u))
        o = None
        for t in range(len(ps)):
            ot = jnp.dot(vb[slot, j, :, t * _CH:(t + 1) * _CH], ps[t],
                         preferred_element_type=jnp.float32) * be[t]
            o = ot if o is None else o + ot
        ob[slot, j, :, c0:c1] = o[:, :c1 - c0].astype(ob.dtype)

    n = len(heads)
    if _ORDER == 'headlook':
        for u in range(nsp):
            QK(heads[0], u)
            SM(heads[0], u)
        for x in range(n):
            if x + 1 < n:
                for u in range(nsp):
                    QK(heads[x + 1], u)
                    SM(heads[x + 1], u)
            else:
                emit_kt_next()
            for u in range(nsp):
                PV(heads[x], u)
    elif _ORDER == 'head':
        for x in range(n):
            for u in range(nsp):
                QK(heads[x], u)
                SM(heads[x], u)
            if x == n - 1:
                emit_kt_next()
            for u in range(nsp):
                PV(heads[x], u)


def _mha_kernel(q_hbm, k_hbm, v_hbm, o_hbm, qb, kb, vb, ob, ktT, k0, sem, rsem, *, scale, NG):
    c = scale * math.log2(math.e)
    G = _G
    NR_IN, NR_OUT = len(_RAMP_IN), len(_RAMP_OUT)
    sh = 1 if _CARRY else 0

    def copies(g, slot, a, b, s_k, s_q, s_v, last=False):
        nk = b - a if not (last and sh) else b - a - 1
        out = []
        if nk > 0:
            out.append(pltpu.make_async_copy(k_hbm.at[pl.ds(g * G + a + sh, nk)], kb.at[slot, pl.ds(a, nk)], s_k))
        out.append(pltpu.make_async_copy(q_hbm.at[pl.ds(g * G + a, b - a)], qb.at[slot, pl.ds(a, b - a)], s_q))
        out.append(pltpu.make_async_copy(v_hbm.at[pl.ds(g * G + a, b - a)], vb.at[slot, pl.ds(a, b - a)], s_v))
        return out

    def group_in(g, slot, last=False):
        return copies(g, slot, 0, G, sem.at[slot * 4], sem.at[slot * 4 + 1], sem.at[slot * 4 + 2], last)

    def group_out(g, slot):
        return pltpu.make_async_copy(ob.at[slot], o_hbm.at[pl.ds(g * G, G)], sem.at[slot * 4 + 3])

    def part_out(g, slot, a, b, s):
        return pltpu.make_async_copy(ob.at[slot, pl.ds(a, b - a)], o_hbm.at[pl.ds(g * G + a, b - a)], s)

    def segment(slot, a, b, first_kt, write_next):
        kts = {}

        def get_kt(j):
            if j not in kts:
                if _CARRY and j == a:
                    kts[j] = first_kt()
                else:
                    kts[j] = kb[slot, j - sh].T
            return kts[j]

        def emit_kt_next():
            if write_next and _CARRY:
                ktT[...] = kb[slot, b - 1].T

        _compute_heads(list(range(a, b)), get_kt, emit_kt_next, qb, vb, ob, slot, c)

    def bounds(sizes):
        out, a = [], 0
        for s in sizes:
            out.append((a, a + s))
            a += s
        assert a == G
        return out

    rin = bounds(_RAMP_IN)
    rin_cp = [copies(0, 0, a, b, rsem.at[3 * s], rsem.at[3 * s + 1], rsem.at[3 * s + 2], last=(NG == 1 and s == NR_IN - 1))
              for s, (a, b) in enumerate(rin)]
    k0_cp = pltpu.make_async_copy(k_hbm.at[0], k0, rsem.at[3 * NR_IN])
    if _CARRY:
        k0_cp.start()
    for s in range(min(2, NR_IN)):
        for cp in rin_cp[s]:
            cp.start()
    if NR_IN < 2:
        for cp in group_in(1, 1):
            cp.start()
    for s, (a, b) in enumerate(rin):
        if s == 0 and _CARRY:
            k0_cp.wait()
        for cp in rin_cp[s]:
            cp.wait()
        if s + 2 < NR_IN:
            for cp in rin_cp[s + 2]:
                cp.start()
        elif s + 2 == NR_IN:
            for cp in group_in(1, 1, last=(NG == 2)):
                cp.start()
        segment(0, a, b, (lambda: k0[...].T) if s == 0 else (lambda: ktT[...]), True)

    def body(g, carry):
        slot = lax.rem(g, 2)
        nslot = 1 - slot

        @pl.when(g + 2 < NG)
        def _():
            for cp in group_in(g + 1, nslot):
                cp.start()

        @pl.when(g + 2 == NG)
        def _():
            for cp in group_in(g + 1, nslot, last=True):
                cp.start()

        group_out(g - 1, nslot).start()
        for cp in group_in(g, slot):
            cp.wait()

        @pl.when(g >= 2)
        def _():
            group_out(g - 2, slot).wait()

        segment(slot, 0, G, lambda: ktT[...], True)
        return carry

    lax.fori_loop(1, NG - 1, body, 0)

    gl = NG - 1
    sl = gl % 2
    group_out(gl - 1, 1 - sl).start()
    for cp in group_in(gl, sl, last=True):
        cp.wait()
    if gl >= 2:
        group_out(gl - 2, sl).wait()
    rout = bounds(_RAMP_OUT)
    for s, (a, b) in enumerate(rout):
        segment(sl, a, b, lambda: ktT[...], s + 1 < NR_OUT)
        part_out(gl, sl, a, b, rsem.at[3 * NR_IN + 1 + s]).start()
    group_out(gl - 1, 1 - sl).wait()
    for s, (a, b) in enumerate(rout):
        part_out(gl, sl, a, b, rsem.at[3 * NR_IN + 1 + s]).wait()


@jax.jit
def pallas_standalone__mha_softmax__near_ridge_kernel(q, k, v):
    B, H, Sq, D = q.shape
    Sk = k.shape[2]
    scale = float(D) ** -0.5
    qt = jnp.swapaxes(q, 2, 3).reshape(B * H, D, Sq)
    kt = jnp.swapaxes(k, 2, 3).reshape(B * H, D, Sk)
    vt = jnp.swapaxes(v, 2, 3).reshape(B * H, D, Sk)
    G = _G
    NG = B * H // G
    ot = pl.pallas_call(
        functools.partial(_mha_kernel, scale=scale, NG=NG),
        in_specs=[pl.BlockSpec(memory_space=pl.ANY)] * 3,
        out_specs=pl.BlockSpec(memory_space=pl.ANY),
        out_shape=jax.ShapeDtypeStruct((B * H, D, Sq), q.dtype),
        scratch_shapes=[
            pltpu.VMEM((2, G, D, Sq), q.dtype),
            pltpu.VMEM((2, G, D, Sk), k.dtype),
            pltpu.VMEM((2, G, D, Sk), v.dtype),
            pltpu.VMEM((2, G, D, Sq), q.dtype),
            pltpu.VMEM((Sk, D), k.dtype),
            pltpu.VMEM((D, Sk), k.dtype),
            pltpu.SemaphoreType.DMA((8,)),
            pltpu.SemaphoreType.DMA((3 * len(_RAMP_IN) + 1 + len(_RAMP_OUT),)),
        ],
        compiler_params=pltpu.CompilerParams(
            vmem_limit_bytes=100 * 1024 * 1024,
            flags=_FLAGS,
            disable_bounds_checks=True,
        ),
    )(qt, kt, vt)
    return jnp.swapaxes(ot.reshape(B, H, D, Sq), 2, 3)
```

```python
import functools
import math

import jax
import jax.numpy as jnp
from jax import lax
import jax.experimental.pallas as pl
import jax.experimental.pallas.tpu as pltpu

_G = 16
_FLAGS = {"XLA_TPU_RESCHEDULE_DMA_DONES": True}
_CH = 128
_W = 512
_ORDER = 'head'
_PAD = True
_NOBC = True
_SG = 2
_CARRY = True
_PRO = 16


def _mha_kernel(q_hbm, k_hbm, v_hbm, o_hbm, qb, kb, vb, ob, ktT, sq, sk, sv, so, *, scale, NH):
    c = scale * math.log2(math.e)
    G = _G
    NG = NH // G
    Sq = qb.shape[-1]
    W = _W
    splits = [(c0, min(c0 + W, Sq)) for c0 in range(0, Sq, W)]
    nsp = len(splits)
    refs = {'q': (q_hbm, qb, sq), 'k': (k_hbm, kb, sk), 'v': (v_hbm, vb, sv)}

    SG = _SG
    assert G % SG == 0

    def in_copy(which, head, slot, j):
        hbm, buf, sem = refs[which]
        return pltpu.make_async_copy(hbm.at[pl.ds(head, SG)], buf.at[slot, pl.ds(j, SG)],
                                     sem.at[(slot * G + j) // SG])

    def out_copy(head, slot, j):
        return pltpu.make_async_copy(ob.at[slot, pl.ds(j, SG)], o_hbm.at[pl.ds(head, SG)],
                                     so.at[(slot * G + j) // SG])

    def pro(i, carry):
        j = i * SG
        in_copy('k', j, 0, j).start()
        in_copy('q', j, 0, j).start()
        in_copy('v', j, 0, j).start()
        return carry
    lax.fori_loop(0, G // SG, pro, 0)
    if _CARRY:
        in_copy('k', 0, 0, 0).wait()
        ktT[...] = kb[0, 0].T

    def body(g, carry):
        slot = lax.rem(g, 2)
        nslot = 1 - slot
        h0 = g * G
        more = g + 1 < NG
        kts = {}
        S = {}
        P = {}

        def get_kt(j):
            if j not in kts:
                if j % SG == 0:
                    if not (_CARRY and j == 0):
                        in_copy('k', h0 + j, slot, j).wait()
                    in_copy('q', h0 + j, slot, j).wait()
                    if _CARRY and j == 0:
                        in_copy('k', jnp.minimum(h0 + G, NH - G), nslot, 0).start()

                        @pl.when(more)
                        def _():
                            in_copy('q', h0 + G + j, nslot, j).start()
                            in_copy('v', h0 + G + j, nslot, j).start()
                    else:
                        @pl.when(more)
                        def _():
                            in_copy('k', h0 + G + j, nslot, j).start()
                            in_copy('q', h0 + G + j, nslot, j).start()
                            in_copy('v', h0 + G + j, nslot, j).start()
                if _CARRY and j == 0:
                    kts[j] = ktT[...]
                else:
                    kts[j] = kb[slot, j].T
            return kts[j]

        def QK(j, u):
            c0, c1 = splits[u]
            kt = get_kt(j)
            qq = qb[slot, j, :, c0:c1]
            if _PAD and c1 - c0 < W:
                qq = jnp.pad(qq, ((0, 0), (0, W - (c1 - c0))))
            S[j, u] = jnp.dot(kt, qq, preferred_element_type=jnp.float32)

        def SM(j, u):
            s = S.pop((j, u))
            nch = s.shape[0] // _CH
            w = s.shape[1]
            ms, ps, ls = [], [], []
            m = None
            for t in range(nch):
                st = s[t * _CH:(t + 1) * _CH] * c
                mt = jnp.max(st, axis=0, keepdims=True)
                m = mt if m is None else jnp.maximum(m, mt)
                p = jnp.exp2(st - m)
                ms.append(m)
                ls.append(jnp.sum(p.reshape(_CH // 8, 8, w), axis=0))
                ps.append(p.astype(jnp.bfloat16))
            al = [jnp.exp2(mm - m) for mm in ms[:-1]]
            l = ls[-1]
            for t in range(nch - 1):
                l = l + al[t] * ls[t]
            l = jnp.sum(l, axis=0, keepdims=True)
            r = 1.0 / l
            P[j, u] = (ps, [a * r for a in al] + [r])

        def PV(j, u):
            c0, c1 = splits[u]
            ps, be = P.pop((j, u))
            if u == 0 and j % SG == 0:
                in_copy('v', h0 + j, slot, j).wait()

                @pl.when(g >= 2)
                def _():
                    out_copy(h0 + j - 2 * G, slot, j).wait()
            o = None
            for t in range(len(ps)):
                ot = jnp.dot(vb[slot, j, :, t * _CH:(t + 1) * _CH], ps[t],
                             preferred_element_type=jnp.float32) * be[t]
                o = ot if o is None else o + ot
            ob[slot, j, :, c0:c1] = o[:, :c1 - c0].astype(ob.dtype)
            if u == nsp - 1 and j % SG == SG - 1:
                out_copy(h0 + j - (SG - 1), slot, j - (SG - 1)).start()

        def next_kt():
            if _CARRY:
                in_copy('k', 0, nslot, 0).wait()
                ktT[...] = kb[nslot, 0].T

        if _ORDER == 'headlook':
            for u in range(nsp):
                QK(0, u)
                SM(0, u)
            for j in range(G):
                if j + 1 < G:
                    for u in range(nsp):
                        QK(j + 1, u)
                        SM(j + 1, u)
                else:
                    next_kt()
                for u in range(nsp):
                    PV(j, u)
        elif _ORDER == 'head':
            for j in range(G):
                for u in range(nsp):
                    QK(j, u)
                    SM(j, u)
                if j == G - 1:
                    next_kt()
                for u in range(nsp):
                    PV(j, u)
        return carry

    lax.fori_loop(0, NG, body, 0)

    for g in range(max(0, NG - 2), NG):
        for j in range(0, G, SG):
            out_copy(g * G + j, g % 2, j).wait()


@jax.jit
def pallas_standalone__mha_softmax__near_ridge_kernel(q, k, v):
    B, H, Sq, D = q.shape
    Sk = k.shape[2]
    scale = float(D) ** -0.5
    qt = jnp.swapaxes(q, 2, 3).reshape(B * H, D, Sq)
    kt = jnp.swapaxes(k, 2, 3).reshape(B * H, D, Sk)
    vt = jnp.swapaxes(v, 2, 3).reshape(B * H, D, Sk)
    G = _G
    ot = pl.pallas_call(
        functools.partial(_mha_kernel, scale=scale, NH=B * H),
        in_specs=[pl.BlockSpec(memory_space=pl.ANY)] * 3,
        out_specs=pl.BlockSpec(memory_space=pl.ANY),
        out_shape=jax.ShapeDtypeStruct((B * H, D, Sq), q.dtype),
        scratch_shapes=[
            pltpu.VMEM((2, G, D, Sq), q.dtype),
            pltpu.VMEM((2, G, D, Sk), k.dtype),
            pltpu.VMEM((2, G, D, Sk), v.dtype),
            pltpu.VMEM((2, G, D, Sq), q.dtype),
            pltpu.VMEM((Sk, D), k.dtype),
            pltpu.SemaphoreType.DMA((2 * G // _SG,)),
            pltpu.SemaphoreType.DMA((2 * G // _SG,)),
            pltpu.SemaphoreType.DMA((2 * G // _SG,)),
            pltpu.SemaphoreType.DMA((2 * G // _SG,)),
        ],
        compiler_params=pltpu.CompilerParams(
            vmem_limit_bytes=100 * 1024 * 1024,
            flags=_FLAGS,
            disable_bounds_checks=_NOBC,
        ),
    )(qt, kt, vt)
    return jnp.swapaxes(ot.reshape(B, H, D, Sq), 2, 3)
```

```python
import functools
import math

import jax
import jax.numpy as jnp
from jax import lax
import jax.experimental.pallas as pl
import jax.experimental.pallas.tpu as pltpu

_G = 32
_FLAGS = {"XLA_TPU_RESCHEDULE_DMA_DONES": True}
_CH = 128
_W = 512
_ORDER = 'head'
_PAD = True
_NOSC = True
_NOBC = True
_R = 32
_L = 16
_RO = 16
_IN_SIZES = (1, 1, 2, 3, 3, 3, 3)
_OUT_SIZES = (4, 4, 4, 2, 1, 1)
_KT_AT = -1
_CARRY = True
_PRO = 16


def _mha_kernel(q_hbm, k_hbm, v_hbm, o_hbm, qb, kb, vb, ob, ktT, si, so, *, scale, NH):
    c = scale * math.log2(math.e)
    G, R, L, RO = _G, _R, _L, _RO
    NG = NH // G
    Sq = qb.shape[-1]
    W = _W
    splits = [(c0, min(c0 + W, Sq)) for c0 in range(0, Sq, W)]
    nsp = len(splits)
    refs = {'k': (k_hbm, kb, 0), 'q': (q_hbm, qb, 1), 'v': (v_hbm, vb, 2)}
    assert G % R == 0 and G % RO == 0 and L < R and NH % G == 0

    def starts(sizes):
        out, a = {}, 0
        for s in sizes:
            out[a] = s
            a += s
        return out

    in_chunk = {p: n for base in range(0, G, L) for (o, n) in starts(_IN_SIZES).items() for p in [base + o]}
    out_chunk = {p: n for base in range(0, G, RO) for (o, n) in starts(_OUT_SIZES).items() for p in [base + o]}
    out_end = {p + n - 1: p for p, n in out_chunk.items()}
    assert sum(_IN_SIZES) == L and sum(_OUT_SIZES) == RO and G % L == 0

    in_id = {p: i for i, p in enumerate(sorted(p for p in in_chunk if p < R))}
    out_id = {p: i for i, p in enumerate(sorted(p for p in out_chunk if p < RO))}

    def in_copy(which, head, j):
        hbm, buf, t = refs[which]
        n = in_chunk[j % G]
        return pltpu.make_async_copy(hbm.at[pl.ds(head, n)], buf.at[pl.ds(j % R, n)], si.at[3 * in_id[j % R] + t])

    def out_copy(head, j):
        n = out_chunk[j]
        return pltpu.make_async_copy(ob.at[pl.ds(j % RO, n)], o_hbm.at[pl.ds(head, n)], so.at[out_id[j % RO]])

    for j in sorted(p for p in in_chunk if p < L):
        for w in ('k', 'q', 'v'):
            in_copy(w, j, j).start()
    in_copy('k', 0, 0).wait()
    ktT[...] = kb[0].T

    def body(g, carry):
        h0 = g * G
        more = g + 1 < NG
        kts = {}
        S = {}
        P = {}

        def get_kt(j):
            if j not in kts:
                if j in in_chunk:
                    if j != 0:
                        in_copy('k', h0 + j, j).wait()
                    in_copy('q', h0 + j, j).wait()
                    if j + L < G:
                        for w in ('k', 'q', 'v'):
                            in_copy(w, h0 + j + L, j + L).start()
                    else:
                        if j + L == G:
                            n = in_chunk[0]
                            in_copy('k', jnp.minimum(h0 + G, NH - n), G).start()
                        else:
                            @pl.when(more)
                            def _():
                                in_copy('k', h0 + j + L, j + L).start()

                        @pl.when(more)
                        def _():
                            in_copy('q', h0 + j + L, j + L).start()
                            in_copy('v', h0 + j + L, j + L).start()
                kts[j] = ktT[...] if j == 0 else kb[j % R].T
            return kts[j]

        def QK(j, u):
            c0, c1 = splits[u]
            kt = get_kt(j)
            qq = qb[j % R, :, c0:c1]
            if _PAD and c1 - c0 < W:
                qq = jnp.pad(qq, ((0, 0), (0, W - (c1 - c0))))
            S[j, u] = jnp.dot(kt, qq, preferred_element_type=jnp.float32)

        def SM(j, u):
            s = S.pop((j, u))
            nch = s.shape[0] // _CH
            w = s.shape[1]
            ms, ps, ls = [], [], []
            m = None
            for t in range(nch):
                st = s[t * _CH:(t + 1) * _CH] * c
                mt = jnp.max(st, axis=0, keepdims=True)
                m = mt if m is None else jnp.maximum(m, mt)
                p = jnp.exp2(st - m)
                ms.append(m)
                ls.append(jnp.sum(p.reshape(_CH // 8, 8, w), axis=0))
                ps.append(p.astype(jnp.bfloat16))
            al = [jnp.exp2(mm - m) for mm in ms[:-1]]
            l = ls[-1]
            for t in range(nch - 1):
                l = l + al[t] * ls[t]
            l = jnp.sum(l, axis=0, keepdims=True)
            r = 1.0 / l
            P[j, u] = (ps, [a * r for a in al] + [r])

        def PV(j, u):
            c0, c1 = splits[u]
            ps, be = P.pop((j, u))
            if u == 0:
                if j in in_chunk:
                    in_copy('v', h0 + j, j).wait()
                if j in out_chunk:
                    if j >= RO:
                        out_copy(h0 + j - RO, j - RO).wait()
                    else:
                        @pl.when(g >= 1)
                        def _():
                            out_copy(h0 + j - RO, G + j - RO).wait()
            o = None
            for t in range(len(ps)):
                ot = jnp.dot(vb[j % R, :, t * _CH:(t + 1) * _CH], ps[t],
                             preferred_element_type=jnp.float32) * be[t]
                o = ot if o is None else o + ot
            ob[j % RO, :, c0:c1] = o[:, :c1 - c0].astype(ob.dtype)
            if u == nsp - 1 and j in out_end:
                out_copy(h0 + out_end[j], out_end[j]).start()

        def next_kt():
            in_copy('k', 0, G).wait()
            ktT[...] = kb[G % R].T

        if _ORDER == 'headlook':
            for u in range(nsp):
                QK(0, u)
                SM(0, u)
            for j in range(G):
                if j + 1 < G:
                    for u in range(nsp):
                        QK(j + 1, u)
                        SM(j + 1, u)
                else:
                    next_kt()
                for u in range(nsp):
                    PV(j, u)
        elif _ORDER == 'head':
            for j in range(G):
                for u in range(nsp):
                    QK(j, u)
                    SM(j, u)
                if j == _KT_AT % G:
                    next_kt()
                for u in range(nsp):
                    PV(j, u)
        return carry

    lax.fori_loop(0, NG, body, 0)

    for j in sorted(p for p in out_chunk if p >= G - RO):
        out_copy((NG - 1) * G + j, j).wait()


@jax.jit
def pallas_standalone__mha_softmax__near_ridge_kernel(q, k, v):
    B, H, Sq, D = q.shape
    Sk = k.shape[2]
    scale = float(D) ** -0.5
    qt = jnp.swapaxes(q, 2, 3).reshape(B * H, D, Sq)
    kt = jnp.swapaxes(k, 2, 3).reshape(B * H, D, Sk)
    vt = jnp.swapaxes(v, 2, 3).reshape(B * H, D, Sk)
    G = _G
    ot = pl.pallas_call(
        functools.partial(_mha_kernel, scale=scale, NH=B * H),
        in_specs=[pl.BlockSpec(memory_space=pl.ANY)] * 3,
        out_specs=pl.BlockSpec(memory_space=pl.ANY),
        out_shape=jax.ShapeDtypeStruct((B * H, D, Sq), q.dtype),
        scratch_shapes=[
            pltpu.VMEM((_R, D, Sq), q.dtype),
            pltpu.VMEM((_R, D, Sk), k.dtype),
            pltpu.VMEM((_R, D, Sk), v.dtype),
            pltpu.VMEM((_RO, D, Sq), q.dtype),
            pltpu.VMEM((Sk, D), k.dtype),
            pltpu.SemaphoreType.DMA((3 * len(_IN_SIZES) * (_R // _L),)),
            pltpu.SemaphoreType.DMA((len(_OUT_SIZES),)),
        ],
        compiler_params=pltpu.CompilerParams(
            vmem_limit_bytes=100 * 1024 * 1024,
            flags=_FLAGS,
            disable_bounds_checks=_NOBC,
            disable_semaphore_checks=_NOSC,
        ),
    )(qt, kt, vt)
    return jnp.swapaxes(ot.reshape(B, H, D, Sq), 2, 3)
```

```python
import functools
import math

import jax
import jax.numpy as jnp
from jax import lax
import jax.experimental.pallas as pl
import jax.experimental.pallas.tpu as pltpu

_LANES = 128
_KEY_TILE = 128
_GROUP = 32
_LEAD = 16
_OUT_RING = 16
_IN_CHUNKS = (1, 1, 2, 3, 3, 3, 3)
_OUT_CHUNKS = (4, 4, 4, 2, 1, 1)


def _chunk_starts(sizes, window, total):
    assert sum(sizes) == window and total % window == 0
    out = {}
    for base in range(0, total, window):
        pos = base
        for n in sizes:
            out[pos] = n
            pos += n
    return out


def _mha_kernel(q_hbm, k_hbm, v_hbm, o_hbm, q_buf, k_buf, v_buf, o_buf, kt_next, in_sems, out_sems,
                *, scale):
    num_heads, _, seq_q = q_hbm.shape
    seq_k = k_hbm.shape[2]
    G, L, RO = _GROUP, _LEAD, _OUT_RING
    num_groups = num_heads // G
    assert num_heads % G == 0 and seq_k % _KEY_TILE == 0
    seq_q_pad = -(-seq_q // _LANES) * _LANES
    num_tiles = seq_k // _KEY_TILE
    c = scale * math.log2(math.e)

    in_chunk = _chunk_starts(_IN_CHUNKS, L, G)
    out_chunk = _chunk_starts(_OUT_CHUNKS, RO, G)
    in_id = {p: i for i, p in enumerate(sorted(in_chunk))}
    out_id = {p: i for i, p in enumerate(sorted(p for p in out_chunk if p < RO))}
    out_last = {p + n - 1: p for p, n in out_chunk.items()}
    sources = {"k": (k_hbm, k_buf, 0), "q": (q_hbm, q_buf, 1), "v": (v_hbm, v_buf, 2)}

    def in_copy(which, head, pos):
        hbm, buf, t = sources[which]
        n = in_chunk[pos]
        return pltpu.make_async_copy(
            hbm.at[pl.ds(head, n)], buf.at[pl.ds(pos, n)], in_sems.at[3 * in_id[pos] + t])

    def out_copy(head, pos):
        n = out_chunk[pos]
        return pltpu.make_async_copy(
            o_buf.at[pl.ds(pos % RO, n)], o_hbm.at[pl.ds(head, n)], out_sems.at[out_id[pos % RO]])

    for pos in sorted(p for p in in_chunk if p < L):
        for which in "kqv":
            in_copy(which, pos, pos).start()
    in_copy("k", 0, 0).wait()
    kt_next[...] = k_buf[0].T

    def group(g, carry):
        h0 = g * G
        has_next = g + 1 < num_groups
        next_k_head = jnp.minimum(h0 + G, num_heads - in_chunk[0])

        def fetch(j):
            if j in in_chunk:
                if j != 0:
                    in_copy("k", h0 + j, j).wait()
                in_copy("q", h0 + j, j).wait()
            pos = (j + L) % G
            if pos not in in_chunk:
                return
            if j + L < G:
                for which in "kqv":
                    in_copy(which, h0 + j + L, pos).start()
                return
            if pos == 0:
                in_copy("k", next_k_head, 0).start()

            @pl.when(has_next)
            def _():
                for which in ("qv" if pos == 0 else "kqv"):
                    in_copy(which, h0 + j + L, pos).start()

        def scores(j):
            k = kt_next[...] if j == 0 else k_buf[j].T
            q_t = q_buf[j]
            if seq_q_pad != seq_q:
                q_t = jnp.pad(q_t, ((0, 0), (0, seq_q_pad - seq_q)))
            return jnp.dot(k, q_t, preferred_element_type=jnp.float32)

        def softmax(s):
            maxes, probs, sums = [], [], []
            m = None
            for t in range(num_tiles):
                st = s[t * _KEY_TILE:(t + 1) * _KEY_TILE] * c
                mt = jnp.max(st, axis=0, keepdims=True)
                m = mt if m is None else jnp.maximum(m, mt)
                p = jnp.exp2(st - m)
                maxes.append(m)
                sums.append(jnp.sum(p.reshape(_KEY_TILE // 8, 8, p.shape[1]), axis=0))
                probs.append(p.astype(jnp.bfloat16))
            alphas = [jnp.exp2(mm - m) for mm in maxes[:-1]]
            l = sums[-1]
            for t in range(num_tiles - 1):
                l = l + alphas[t] * sums[t]
            r = 1.0 / jnp.sum(l, axis=0, keepdims=True)
            return probs, [a * r for a in alphas] + [r]

        def output(j, probs, weights):
            if j in in_chunk:
                in_copy("v", h0 + j, j).wait()
            if j in out_chunk:
                if j >= RO:
                    out_copy(h0 + j - RO, j - RO).wait()
                else:
                    @pl.when(g >= 1)
                    def _():
                        out_copy(h0 + j - RO, G + j - RO).wait()
            o = None
            for t in range(num_tiles):
                v_t = v_buf[j, :, t * _KEY_TILE:(t + 1) * _KEY_TILE]
                part = jnp.dot(v_t, probs[t], preferred_element_type=jnp.float32) * weights[t]
                o = part if o is None else o + part
            o_buf[j % RO] = o[:, :seq_q].astype(o_buf.dtype)
            if j in out_last:
                out_copy(h0 + out_last[j], out_last[j]).start()

        for j in range(G):
            fetch(j)
            probs, weights = softmax(scores(j))
            if j == G - 1:
                in_copy("k", next_k_head, 0).wait()
                kt_next[...] = k_buf[0].T
            output(j, probs, weights)
        return carry

    lax.fori_loop(0, num_groups, group, 0)

    for pos in sorted(p for p in out_chunk if p >= G - RO):
        out_copy((num_groups - 1) * G + pos, pos).wait()


@jax.jit
def pallas_standalone__mha_softmax__near_ridge_kernel(q, k, v):
    B, H, Sq, D = q.shape
    Sk = k.shape[2]
    qt = jnp.swapaxes(q, 2, 3).reshape(B * H, D, Sq)
    kt = jnp.swapaxes(k, 2, 3).reshape(B * H, D, Sk)
    vt = jnp.swapaxes(v, 2, 3).reshape(B * H, D, Sk)
    ot = pl.pallas_call(
        functools.partial(_mha_kernel, scale=float(D) ** -0.5),
        in_specs=[pl.BlockSpec(memory_space=pl.ANY)] * 3,
        out_specs=pl.BlockSpec(memory_space=pl.ANY),
        out_shape=jax.ShapeDtypeStruct((B * H, D, Sq), q.dtype),
        scratch_shapes=[
            pltpu.VMEM((_GROUP, D, Sq), q.dtype),
            pltpu.VMEM((_GROUP, D, Sk), k.dtype),
            pltpu.VMEM((_GROUP, D, Sk), v.dtype),
            pltpu.VMEM((_OUT_RING, D, Sq), q.dtype),
            pltpu.VMEM((Sk, D), k.dtype),
            pltpu.SemaphoreType.DMA((3 * len(_IN_CHUNKS) * (_GROUP // _LEAD),)),
            pltpu.SemaphoreType.DMA((len(_OUT_CHUNKS),)),
        ],
        compiler_params=pltpu.CompilerParams(
            vmem_limit_bytes=48 * 1024 * 1024,
            flags={"XLA_TPU_RESCHEDULE_DMA_DONES": True},
            disable_bounds_checks=True,
            disable_semaphore_checks=True,
        ),
    )(qt, kt, vt)
    return jnp.swapaxes(ot.reshape(B, H, D, Sq), 2, 3)
```
